```python
import os as _os
_os.environ.setdefault("JAX_PLATFORMS", "cpu")
import jax
import jax.numpy as jnp

def _softmax(x, axis=-1):
    return jax.nn.softmax(x, axis=axis)
def _gelu(x):
    return jax.nn.gelu(x, approximate=True)
def _silu(x):
    return jax.nn.silu(x)
def _sigmoid(x):
    return jax.nn.sigmoid(x)
def _layernorm(x, axis=-1, eps=1e-5):
    m = jnp.mean(x, axis=axis, keepdims=True)
    v = jnp.var(x, axis=axis, keepdims=True)
    return (x - m) / jnp.sqrt(v + eps)
def _scatter_add(tgt, idx, src, axis=0):
    return tgt.at[idx].add(src)
def _segment_sum(src, seg, n):
    return jax.ops.segment_sum(src, seg, n)
class _Rng:
    def __init__(self, key):
        self._k = key
    def _next(self):
        self._k, sub = jax.random.split(self._k)
        return sub
    def normal(self, shape):
        return jax.random.normal(self._next(), shape, dtype=jnp.bfloat16)
    def randint(self, lo, hi, shape):
        return jax.random.randint(self._next(), shape, lo, hi, dtype=jnp.int32)
    def uniform(self, shape, lo=0.0, hi=1.0):
        return jax.random.uniform(self._next(), shape, jnp.bfloat16, lo, hi)
    def permutation(self, n):
        return jax.random.permutation(self._next(), n)


kernel_name = 'standalone__mha_softmax__near_ridge'

def setup_inputs():
    _rng = _Rng(jax.random.key(int.from_bytes(__import__("os").urandom(4), "little")))
    _w = (lambda a: (lambda t: t.astype(jnp.bfloat16) if jnp.issubdtype(t.dtype, jnp.floating) else t)(jnp.asarray(a)))
    B, H, Sq, Sk, D = 8, 32, 496, 512, 192
    return {
        "q": _w((lambda *s: _rng.normal(s) * 0.05)(B, H, Sq, D)),
        "k": _w((lambda *s: _rng.normal(s) * 3.2)(B, H, Sk, D)),
        "v": _w((lambda *s: _rng.normal(s) * 0.05)(B, H, Sk, D)),
    }

def reference(q, k, v):
    scale = q.shape[-1] ** -0.5
    scores = jnp.einsum("bhqd,bhkd->bhqk", q, k) * scale
    p = _softmax(scores, axis=-1)
    return jnp.einsum("bhqk,bhkd->bhqd", p, v)
```

```python
import math

import jax
import jax.numpy as jnp
import jax.experimental.pallas as pl
import jax.experimental.pallas.tpu as pltpu


@jax.jit
def pallas_standalone__mha_softmax__near_ridge_kernel(
    q: jax.Array,
    k: jax.Array,
    v: jax.Array,
):
    B, H, Sq, D = q.shape
    Sk = k.shape[2]
    hb = 8
    c = (D ** -0.5) * math.log2(math.e)

    qt = jnp.swapaxes(q, 2, 3).reshape(B * H, D, Sq)
    kt = jnp.swapaxes(k, 2, 3).reshape(B * H, D, Sk)
    vt = jnp.swapaxes(v, 2, 3).reshape(B * H, D, Sk)

    def kernel(q_ref, k_ref, v_ref, o_ref):
        def qk(h):
            return jax.lax.dot_general(
                k_ref[h], q_ref[h], (((0,), (0,)), ((), ())),
                preferred_element_type=jnp.float32)

        s_next = qk(0)
        for h in range(hb):
            st = s_next
            if h + 1 < hb:
                s_next = qk(h + 1)
            m = jnp.max(st, axis=0, keepdims=True)
            p = jnp.exp2((st - m) * c)
            l = jnp.sum(p, axis=0, keepdims=True)
            ot = jnp.dot(v_ref[h], p.astype(jnp.bfloat16), preferred_element_type=jnp.float32)
            o_ref[h] = (ot * (1.0 / l)).astype(o_ref.dtype)

    ot = pl.pallas_call(
        kernel,
        grid=(B * H // hb,),
        in_specs=[
            pl.BlockSpec((hb, D, Sq), lambda i: (i, 0, 0)),
            pl.BlockSpec((hb, D, Sk), lambda i: (i, 0, 0)),
            pl.BlockSpec((hb, D, Sk), lambda i: (i, 0, 0)),
        ],
        out_specs=pl.BlockSpec((hb, D, Sq), lambda i: (i, 0, 0)),
        out_shape=jax.ShapeDtypeStruct((B * H, D, Sq), q.dtype),
        compiler_params=pltpu.CompilerParams(
            dimension_semantics=("parallel",),
            vmem_limit_bytes=64 * 1024 * 1024,
            flags={"XLA_TPU_FORCE_LP_LLO_SCHEDULER": True},
        ),
    )(qt, kt, vt)
    return jnp.swapaxes(ot.reshape(B, H, D, Sq), 2, 3)
```

```python
import math

import jax
import jax.numpy as jnp
from jax import lax
import jax.experimental.pallas as pl
import jax.experimental.pallas.tpu as pltpu


@jax.jit
def pallas_standalone__mha_softmax__near_ridge_kernel(
    q: jax.Array,
    k: jax.Array,
    v: jax.Array,
):
    B, H, Sq, D = q.shape
    Sk = k.shape[2]
    NH = B * H
    G = 32
    NB = 4
    NCH = 4
    A0, A1 = 48, 240
    c = (D ** -0.5) * math.log2(math.e)

    qt = jnp.swapaxes(q, 2, 3).reshape(NH, D, Sq)
    kt = jnp.swapaxes(k, 2, 3).reshape(NH, D, Sk)
    vt = jnp.swapaxes(v, 2, 3).reshape(NH, D, Sk)
    cols = [(a, min(a + 128, Sq)) for a in range(0, Sq, 128)]

    def kernel(q_hbm, k_hbm, v_hbm, o_hbm, qb, kb, vb, ob, sq, sk, sv, so):
        def cp_in(src, h, dst, sem, slot):
            return pltpu.make_async_copy(src.at[h], dst.at[slot], sem.at[slot])

        def cp_out(h, slot):
            return pltpu.make_async_copy(ob.at[slot], o_hbm.at[h], so.at[slot])

        for s in range(NB):
            cp_in(q_hbm, s, qb, sq, s).start()
            cp_in(k_hbm, s, kb, sk, s).start()
            cp_in(v_hbm, s, vb, sv, s).start()
        for s in range(NB):
            pltpu.make_async_copy(q_hbm.at[s], ob.at[s], so.at[s]).start()

        def body(g, carry):
            base = g * G
            zero = lax.shift_right_logical(g, 24)

            def dep(x8, anchor):
                a = pltpu.bitcast(anchor, jnp.int32) & jnp.full(x8.shape, zero, jnp.int32)
                return pltpu.bitcast(pltpu.bitcast(x8, jnp.int32) | a, jnp.float32)

            def clamp(h):
                return jnp.minimum(h, NH - 1)

            def waits_qk(j):
                s = j % NB
                cp_in(q_hbm, 0, qb, sq, s).wait()
                cp_in(k_hbm, 0, kb, sk, s).wait()

            def waits_vo(j):
                s = j % NB
                cp_in(v_hbm, 0, vb, sv, s).wait()
                cp_out(0, s).wait()

            def qk(j):
                s = j % NB
                st = lax.dot_general(kb[s], qb[s], (((0,), (0,)), ((), ())),
                                     preferred_element_type=jnp.float32)
                hn = clamp(base + j + NB)
                cp_in(q_hbm, hn, qb, sq, s).start()
                cp_in(k_hbm, hn, kb, sk, s).start()
                return st

            def sm_pv(j, st, st_next):
                s = j % NB
                m = jnp.max(st, axis=0, keepdims=True)
                vv = vb[s]
                outs = []
                rows = Sk // NCH
                step = (D // NCH) // 8 * 8
                for n, (a, b) in enumerate(cols):
                    w = b - a
                    m8 = jnp.broadcast_to(m[:, a:b], (8, w))
                    ps = []
                    lacc = None
                    for i in range(NCH):
                        if n < 2:
                            av = None
                            if st_next is not None:
                                r = (A0 if n == 0 else A1) + i * step
                                av = st_next[r:r + 8, 256:384]
                        else:
                            r = i * step
                            av = outs[n - 2][r:r + 8, 0:128]
                        mi = m8 if av is None else dep(m8, av[:, :w])
                        x = st[i * rows:(i + 1) * rows, a:b].reshape(rows // 8, 8, w) - mi[None]
                        p = jnp.exp2(x * c)
                        ls = jnp.sum(p, axis=0)
                        lacc = ls if lacc is None else lacc + ls
                        ps.append(p.reshape(rows, w))
                    l = jnp.sum(lacc, axis=0, keepdims=True)
                    ot = jnp.dot(vv, jnp.concatenate(ps, axis=0).astype(jnp.bfloat16),
                                 preferred_element_type=jnp.float32)
                    outs.append(ot)
                    ob[s, :, a:b] = (ot * (1.0 / l)).astype(ob.dtype)
                cp_in(v_hbm, clamp(base + j + NB), vb, sv, s).start()
                cp_out(base + j, s).start()
                if j + 2 < G:
                    waits_qk(j + 2)
                if j + 1 < G:
                    waits_vo(j + 1)

            waits_qk(0)
            waits_qk(1)
            waits_vo(0)
            s_next = qk(0)
            for j in range(G):
                st = s_next
                s_next = qk(j + 1) if j + 1 < G else None
                sm_pv(j, st, s_next)
            return carry

        lax.fori_loop(0, NH // G, body, 0)
        for s in range(NB):
            cp_in(q_hbm, 0, qb, sq, s).wait()
            cp_in(k_hbm, 0, kb, sk, s).wait()
            cp_in(v_hbm, 0, vb, sv, s).wait()
            cp_out(0, s).wait()

    ot = pl.pallas_call(
        kernel,
        grid=(1,),
        in_specs=[pl.BlockSpec(memory_space=pl.ANY)] * 3,
        out_specs=pl.BlockSpec(memory_space=pl.ANY),
        out_shape=jax.ShapeDtypeStruct((NH, D, Sq), q.dtype),
        scratch_shapes=[
            pltpu.VMEM((NB, D, Sq), q.dtype),
            pltpu.VMEM((NB, D, Sk), q.dtype),
            pltpu.VMEM((NB, D, Sk), q.dtype),
            pltpu.VMEM((NB, D, Sq), q.dtype),
            pltpu.SemaphoreType.DMA((NB,)),
            pltpu.SemaphoreType.DMA((NB,)),
            pltpu.SemaphoreType.DMA((NB,)),
            pltpu.SemaphoreType.DMA((NB,)),
        ],
        compiler_params=pltpu.CompilerParams(
            dimension_semantics=("arbitrary",),
            vmem_limit_bytes=64 * 1024 * 1024,
            flags={"XLA_TPU_FORCE_LP_LLO_SCHEDULER": True, "XLA_TPU_RESCHEDULE_DMA_DONES": True},
        ),
    )(qt, kt, vt)
    return jnp.swapaxes(ot.reshape(B, H, D, Sq), 2, 3)
```

```python
import math

import jax
import jax.numpy as jnp
from jax import lax
import jax.experimental.pallas as pl
import jax.experimental.pallas.tpu as pltpu


@jax.jit
def pallas_standalone__mha_softmax__near_ridge_kernel(
    q: jax.Array,
    k: jax.Array,
    v: jax.Array,
):
    B, H, Sq, D = q.shape
    Sk = k.shape[2]
    NH = B * H
    G = 32
    NB = 4
    NG = NH // G
    NT = Sq // 128
    QL = Sq - NT * 128
    assert NH % G == 0 and G % NB == 0 and NT == 3 and QL % 16 == 0 and Sk == 512
    c = (D ** -0.5) * math.log2(math.e)
    dn_t = (((0,), (0,)), ((), ()))
    dn_nt = (((1,), (1,)), ((), ()))

    NCH, NSTEP, LEADS = 4, 48, (330, 350, 340)
    CCH, CSTEP, CLEAD = 7, 28, 400
    LAT, DR = 125, 16

    qt = jnp.swapaxes(q, 2, 3).reshape(NH, D, Sq)
    kt = jnp.swapaxes(k, 2, 3).reshape(NH, D, Sk)
    vt = jnp.swapaxes(v, 2, 3).reshape(NH, D, Sk)

    def kernel(q_hbm, k_hbm, v_hbm, o_hbm, qb, kb, vb, ob, sq, sk, sv, so):
        def cp_in(src, h, dst, sem, slot):
            return pltpu.make_async_copy(src.at[h], dst.at[slot], sem.at[slot])

        def cp_out(h, slot):
            return pltpu.make_async_copy(ob.at[slot], o_hbm.at[h], so.at[slot])

        cp_in(k_hbm, 0, kb, sk, 0).start()
        cp_in(q_hbm, 0, qb, sq, 0).start()
        for s in range(1, NB):
            cp_in(k_hbm, s, kb, sk, s).start()
            cp_in(q_hbm, s, qb, sq, s).start()
            cp_in(v_hbm, s - 1, vb, sv, s - 1).start()
        cp_in(v_hbm, NB - 1, vb, sv, NB - 1).start()

        def body(g, carry):
            base = g * G
            zero = lax.shift_right_logical(g, 24)
            not_first = g > 0
            not_last = g < NG - 1

            def dep(x8, anchor):
                a = pltpu.bitcast(anchor, jnp.int32) & jnp.full(x8.shape, zero, jnp.int32)
                return pltpu.bitcast(pltpu.bitcast(x8, jnp.int32) | a, jnp.float32)

            def pad128(av):
                return av if av.shape[1] == 128 else jnp.pad(av, ((0, 0), (0, 128 - av.shape[1])))

            def waits_qk(j):
                s = j % NB
                cp_in(k_hbm, 0, kb, sk, s).wait()
                cp_in(q_hbm, 0, qb, sq, s).wait()

            def waits_vo(j):
                s = j % NB
                cp_in(v_hbm, 0, vb, sv, s).wait()
                if j >= NB:
                    cp_out(0, s).wait()
                else:
                    @pl.when(not_first)
                    def _():
                        cp_out(0, s).wait()

            def maybe(j, f):
                if j + NB < G:
                    f()
                else:
                    pl.when(not_last)(f)

            def start_kq(j):
                s = j % NB

                def f():
                    cp_in(k_hbm, base + j + NB, kb, sk, s).start()
                    cp_in(q_hbm, base + j + NB, qb, sq, s).start()
                maybe(j, f)

            def qk(j):
                s = j % NB
                kk = kb[s]
                qq = qb[s]
                sa = lax.dot_general(kk, qq[:, 0:256], dn_t, preferred_element_type=jnp.float32)
                sb1 = lax.dot_general(kk[:, 0:256], qq[:, 256:384], dn_t, preferred_element_type=jnp.float32)
                sb2 = lax.dot_general(kk[:, 256:512], qq[:, 256:384], dn_t, preferred_element_type=jnp.float32)
                sc = lax.dot_general(qq[:, 384:Sq], kk, dn_t, preferred_element_type=jnp.float32)
                if j == 0:
                    start_kq(j)
                return sa, jnp.concatenate([sb1, sb2], axis=0), sc

            def pick(t_want, nxt, prev, outs):
                cands = []
                if nxt is not None:
                    cands += [(-(480 + 512) + LAT + 8 * i, ("A", i)) for i in range(Sk // 8)]
                    cands += [(-480 + LAT + 8 * i, ("B", i)) for i in range(Sk // 16)]
                    cands += [(-2 * QL + LAT + 8 * i, ("C1", i)) for i in range(QL // 8)]
                    cands += [(-QL + LAT + 8 * i, ("C2", i)) for i in range(QL // 8)]
                elif prev is not None:
                    for n in range(NT + 1):
                        cands += [(D * (n - 4) + LAT + 8 * i, ("p", n, i)) for i in range(D // 8)]
                for n in range(len(outs)):
                    cands += [(D * n + LAT + 8 * i, ("o", n, i)) for i in range(D // 8)]
                if not cands:
                    return None
                w = min(cands, key=lambda x: abs(x[0] - t_want))[1]
                if w[0] == "A":
                    return nxt[0][8 * w[1]:8 * w[1] + 8, 128:256]
                if w[0] == "B":
                    return nxt[1][8 * w[1]:8 * w[1] + 8, :]
                if w[0] == "C1":
                    return nxt[2][8 * w[1]:8 * w[1] + 8, 0:128]
                if w[0] == "C2":
                    return nxt[2][8 * w[1]:8 * w[1] + 8, 384:512]
                if w[0] == "p":
                    return pad128(prev[w[1]][8 * w[2]:8 * w[2] + 8, :])
                return pad128(outs[w[1]][8 * w[2]:8 * w[2] + 8, :])

            def softmax_rows(sc, anchors):
                mc = jnp.max(sc, axis=1, keepdims=True)
                rows = QL // CCH
                ps = []
                for i in range(CCH):
                    r, r2 = i * rows, (i + 1) * rows
                    x = sc[r:r2] - mc[r:r2]
                    if anchors[i] is not None:
                        cd = dep(jnp.full((8, 128), c, jnp.float32), anchors[i])
                        cd4 = jnp.concatenate([cd] * (Sk // 128), axis=1)
                        x = (x.reshape(rows // 8, 8, Sk) * cd4[None]).reshape(rows, Sk)
                    else:
                        x = x * c
                    p = jnp.exp2(x)
                    l = jnp.sum(p, axis=1, keepdims=True)
                    inv = pl.reciprocal(l, approx=True)
                    inv = inv * (2.0 - l * inv)
                    ps.append(p * inv)
                return jnp.concatenate(ps, axis=0).astype(jnp.bfloat16)

            def sm_pv(j, cur, nxt, prev):
                s = j % NB
                sta, stb, sc = cur
                vv = vb[s]
                outs = []
                rows = Sk // NCH
                for n in range(NT):
                    st = sta[:, n * 128:(n + 1) * 128] if n < 2 else stb
                    m8 = jnp.broadcast_to(jnp.max(st, axis=0, keepdims=True), (8, 128))
                    ps = []
                    lacc = None
                    for i in range(NCH):
                        av = pick(D * n - LEADS[n] + i * NSTEP, nxt, prev, outs)
                        mi = m8 if av is None else dep(m8, av)
                        x = st[i * rows:(i + 1) * rows].reshape(rows // 8, 8, 128) - mi[None]
                        p = jnp.exp2(x * c)
                        ls = jnp.sum(p, axis=0)
                        lacc = ls if lacc is None else lacc + ls
                        ps.append(p.reshape(rows, 128))
                    l = jnp.sum(lacc, axis=0, keepdims=True)
                    ot = jnp.dot(vv, jnp.concatenate(ps, axis=0).astype(jnp.bfloat16),
                                 preferred_element_type=jnp.float32)
                    outs.append(ot)
                    ob[s, :, n * 128:(n + 1) * 128] = (ot * (1.0 / l)).astype(ob.dtype)
                anchors = [pick(D * NT - CLEAD + i * CSTEP, nxt, prev, outs) for i in range(CCH)]
                plast = softmax_rows(sc, anchors)
                ot = lax.dot_general(vv, plast, dn_nt, preferred_element_type=jnp.float32)
                outs.append(ot)
                ob[s, :, NT * 128:Sq] = ot.astype(ob.dtype)

                av16 = outs[2][DR:DR + 16, :].astype(jnp.bfloat16)
                vb[s, 0:16, 0:128] = av16
                if j + 1 < G:
                    kb[(j + 1) % NB, 0:16, 0:128] = av16
                    qb[(j + 1) % NB, 0:16, 0:128] = av16
                    start_kq(j + 1)
                maybe(j, lambda: cp_in(v_hbm, base + j + NB, vb, sv, s).start())
                cp_out(base + j, s).start()
                if j + 3 < G:
                    waits_qk(j + 3)
                if j + 1 < G:
                    waits_vo(j + 1)
                return outs

            waits_qk(0)
            s_next = qk(0)
            waits_qk(1)
            waits_qk(2)
            waits_vo(0)
            prev = None
            for j in range(G):
                cur = s_next
                s_next = qk(j + 1) if j + 1 < G else None
                prev = sm_pv(j, cur, s_next, prev)
            return carry

        lax.fori_loop(0, NG, body, 0)
        for s in range(NB):
            cp_out(0, s).wait()

    ot = pl.pallas_call(
        kernel,
        grid=(1,),
        in_specs=[pl.BlockSpec(memory_space=pl.ANY)] * 3,
        out_specs=pl.BlockSpec(memory_space=pl.ANY),
        out_shape=jax.ShapeDtypeStruct((NH, D, Sq), q.dtype),
        scratch_shapes=[
            pltpu.VMEM((NB, D, Sq), q.dtype),
            pltpu.VMEM((NB, D, Sk), k.dtype),
            pltpu.VMEM((NB, D, Sk), v.dtype),
            pltpu.VMEM((NB, D, Sq), q.dtype),
            pltpu.SemaphoreType.DMA((NB,)),
            pltpu.SemaphoreType.DMA((NB,)),
            pltpu.SemaphoreType.DMA((NB,)),
            pltpu.SemaphoreType.DMA((NB,)),
        ],
        compiler_params=pltpu.CompilerParams(
            dimension_semantics=("arbitrary",),
            vmem_limit_bytes=64 * 1024 * 1024,
            flags={"XLA_TPU_FORCE_LP_LLO_SCHEDULER": True, "XLA_TPU_RESCHEDULE_DMA_DONES": True},
        ),
    )(qt, kt, vt)
    return jnp.swapaxes(ot.reshape(B, H, D, Sq), 2, 3)
```

```python
import math

import jax
import jax.numpy as jnp
from jax import lax
import jax.experimental.pallas as pl
import jax.experimental.pallas.tpu as pltpu


@jax.jit
def pallas_standalone__mha_softmax__near_ridge_kernel(
    q: jax.Array,
    k: jax.Array,
    v: jax.Array,
):
    B, H, Sq, D = q.shape
    Sk = k.shape[2]
    NH = B * H
    G = 32
    NB = 4
    NG = NH // G
    NT = Sq // 128
    QL = Sq - NT * 128
    assert NH % G == 0 and G % NB == 0 and NT == 3 and QL % 16 == 0 and Sk == 512
    c = (D ** -0.5) * math.log2(math.e)
    dn_t = (((0,), (0,)), ((), ()))
    dn_nt = (((1,), (1,)), ((), ()))

    NCH, NSTEP, LEADS = 4, 48, (360, 380, 340)
    CCH, CSTEP, CLEAD = 7, 28, 400
    LAT, DR = 125, 32

    qt = jnp.swapaxes(q, 2, 3).reshape(NH, D, Sq)
    kt = jnp.swapaxes(k, 2, 3).reshape(NH, D, Sk)
    vt = jnp.swapaxes(v, 2, 3).reshape(NH, D, Sk)

    def kernel(q_hbm, k_hbm, v_hbm, o_hbm, qb, kb, vb, ob, sq, sk, sv, so):
        def cp_in(src, h, dst, sem, slot):
            return pltpu.make_async_copy(src.at[h], dst.at[slot], sem.at[slot])

        def cp_out(h, slot):
            return pltpu.make_async_copy(ob.at[slot], o_hbm.at[h], so.at[slot])

        cp_in(k_hbm, 0, kb, sk, 0).start()
        cp_in(q_hbm, 0, qb, sq, 0).start()
        for s in range(1, NB):
            cp_in(k_hbm, s, kb, sk, s).start()
            cp_in(q_hbm, s, qb, sq, s).start()
            cp_in(v_hbm, s - 1, vb, sv, s - 1).start()
        cp_in(v_hbm, NB - 1, vb, sv, NB - 1).start()

        def body(g, carry):
            base = g * G
            zero = lax.shift_right_logical(g, 24)
            not_first = g > 0
            not_last = g < NG - 1

            def dep(x8, anchor):
                a = pltpu.bitcast(anchor, jnp.int32) & jnp.full(x8.shape, zero, jnp.int32)
                return pltpu.bitcast(pltpu.bitcast(x8, jnp.int32) | a, jnp.float32)

            def pad128(av):
                return av if av.shape[1] == 128 else jnp.pad(av, ((0, 0), (0, 128 - av.shape[1])))

            def waits_qk(j):
                s = j % NB
                cp_in(k_hbm, 0, kb, sk, s).wait()
                cp_in(q_hbm, 0, qb, sq, s).wait()

            def waits_vo(j):
                s = j % NB
                cp_in(v_hbm, 0, vb, sv, s).wait()
                if j >= NB:
                    cp_out(0, s).wait()
                else:
                    @pl.when(not_first)
                    def _():
                        cp_out(0, s).wait()

            def maybe(j, f):
                if j + NB < G:
                    f()
                else:
                    pl.when(not_last)(f)

            def start_kq(j):
                s = j % NB

                def f():
                    cp_in(k_hbm, base + j + NB, kb, sk, s).start()
                    cp_in(q_hbm, base + j + NB, qb, sq, s).start()
                maybe(j, f)

            def qk(j):
                s = j % NB
                kk = kb[s]
                qq = qb[s]
                sc = lax.dot_general(qq[:, 384:Sq], kk, dn_t, preferred_element_type=jnp.float32)
                sb1 = lax.dot_general(kk[:, 0:256], qq[:, 256:384], dn_t, preferred_element_type=jnp.float32)
                sb2 = lax.dot_general(kk[:, 256:512], qq[:, 256:384], dn_t, preferred_element_type=jnp.float32)
                sa = lax.dot_general(kk, qq[:, 0:256], dn_t, preferred_element_type=jnp.float32)
                if j == 0:
                    start_kq(j)
                return sa, jnp.concatenate([sb1, sb2], axis=0), sc

            def pick(t_want, nxt, prev, outs):
                cands = []
                if nxt is not None:
                    t_c, t_b, t_a = -(2 * QL + 256 + 512), -(256 + 512), -512
                    cands += [(t_c + LAT + 8 * i, ("C1", i)) for i in range(QL // 8)]
                    cands += [(t_c + QL + LAT + 8 * i, ("C2", i)) for i in range(QL // 8)]
                    cands += [(t_b + LAT + 8 * i, ("B", i)) for i in range(Sk // 16)]
                    cands += [(t_a + LAT + 8 * i, ("A", i)) for i in range(Sk // 8)]
                elif prev is not None:
                    for n in range(NT + 1):
                        cands += [(D * (n - 4) + LAT + 8 * i, ("p", n, i)) for i in range(D // 8)]
                for n in range(len(outs)):
                    cands += [(D * n + LAT + 8 * i, ("o", n, i)) for i in range(D // 8)]
                if not cands:
                    return None
                w = min(cands, key=lambda x: abs(x[0] - t_want))[1]
                if w[0] == "A":
                    return nxt[0][8 * w[1]:8 * w[1] + 8, 128:256]
                if w[0] == "B":
                    return nxt[1][8 * w[1]:8 * w[1] + 8, :]
                if w[0] == "C1":
                    return nxt[2][8 * w[1]:8 * w[1] + 8, 0:128]
                if w[0] == "C2":
                    return nxt[2][8 * w[1]:8 * w[1] + 8, 384:512]
                if w[0] == "p":
                    return pad128(prev[w[1]][8 * w[2]:8 * w[2] + 8, :])
                return pad128(outs[w[1]][8 * w[2]:8 * w[2] + 8, :])

            def softmax_rows(sc, anchors):
                mc = jnp.max(sc, axis=1, keepdims=True)
                rows = QL // CCH
                ps = []
                for i in range(CCH):
                    r, r2 = i * rows, (i + 1) * rows
                    x = sc[r:r2] - mc[r:r2]
                    if anchors[i] is not None:
                        cd = dep(jnp.full((8, 128), c, jnp.float32), anchors[i])
                        cd4 = jnp.concatenate([cd] * (Sk // 128), axis=1)
                        x = (x.reshape(rows // 8, 8, Sk) * cd4[None]).reshape(rows, Sk)
                    else:
                        x = x * c
                    p = jnp.exp2(x)
                    l = jnp.sum(p, axis=1, keepdims=True)
                    inv = pl.reciprocal(l, approx=True)
                    inv = inv * (2.0 - l * inv)
                    ps.append(p * inv)
                return jnp.concatenate(ps, axis=0).astype(jnp.bfloat16)

            def sm_pv(j, cur, nxt, prev):
                s = j % NB
                sta, stb, sc = cur
                vv = vb[s]
                outs = []
                rows = Sk // NCH
                for n in range(NT):
                    st = sta[:, n * 128:(n + 1) * 128] if n < 2 else stb
                    m8 = jnp.broadcast_to(jnp.max(st, axis=0, keepdims=True), (8, 128))
                    ps = []
                    lacc = None
                    for i in range(NCH):
                        av = pick(D * n - LEADS[n] + i * NSTEP, nxt, prev, outs)
                        mi = m8 if av is None else dep(m8, av)
                        x = st[i * rows:(i + 1) * rows].reshape(rows // 8, 8, 128) - mi[None]
                        p = jnp.exp2(x * c)
                        ls = jnp.sum(p, axis=0)
                        lacc = ls if lacc is None else lacc + ls
                        ps.append(p.reshape(rows, 128))
                    l = jnp.sum(lacc, axis=0, keepdims=True)
                    ot = jnp.dot(vv, jnp.concatenate(ps, axis=0).astype(jnp.bfloat16),
                                 preferred_element_type=jnp.float32)
                    outs.append(ot)
                    ob[s, :, n * 128:(n + 1) * 128] = (ot * (1.0 / l)).astype(ob.dtype)
                anchors = [pick(D * NT - CLEAD + i * CSTEP, nxt, prev, outs) for i in range(CCH)]
                plast = softmax_rows(sc, anchors)
                ot = lax.dot_general(vv, plast, dn_nt, preferred_element_type=jnp.float32)
                outs.append(ot)
                ob[s, :, NT * 128:Sq] = ot.astype(ob.dtype)

                av16 = outs[2][DR:DR + 16, :].astype(jnp.bfloat16)
                vb[s, 0:16, 0:128] = av16
                if j + 1 < G:
                    kb[(j + 1) % NB, 0:16, 0:128] = av16
                    qb[(j + 1) % NB, 0:16, 0:128] = av16
                    start_kq(j + 1)
                maybe(j, lambda: cp_in(v_hbm, base + j + NB, vb, sv, s).start())
                cp_out(base + j, s).start()
                if j + 3 < G:
                    waits_qk(j + 3)
                if j + 1 < G:
                    waits_vo(j + 1)
                return outs

            waits_qk(0)
            s_next = qk(0)
            waits_qk(1)
            waits_qk(2)
            waits_vo(0)
            prev = None
            for j in range(G):
                cur = s_next
                s_next = qk(j + 1) if j + 1 < G else None
                prev = sm_pv(j, cur, s_next, prev)
            return carry

        lax.fori_loop(0, NG, body, 0)
        for s in range(NB):
            cp_out(0, s).wait()

    ot = pl.pallas_call(
        kernel,
        grid=(1,),
        in_specs=[pl.BlockSpec(memory_space=pl.ANY)] * 3,
        out_specs=pl.BlockSpec(memory_space=pl.ANY),
        out_shape=jax.ShapeDtypeStruct((NH, D, Sq), q.dtype),
        scratch_shapes=[
            pltpu.VMEM((NB, D, Sq), q.dtype),
            pltpu.VMEM((NB, D, Sk), k.dtype),
            pltpu.VMEM((NB, D, Sk), v.dtype),
            pltpu.VMEM((NB, D, Sq), q.dtype),
            pltpu.SemaphoreType.DMA((NB,)),
            pltpu.SemaphoreType.DMA((NB,)),
            pltpu.SemaphoreType.DMA((NB,)),
            pltpu.SemaphoreType.DMA((NB,)),
        ],
        compiler_params=pltpu.CompilerParams(
            dimension_semantics=("arbitrary",),
            vmem_limit_bytes=64 * 1024 * 1024,
            flags={"XLA_TPU_FORCE_LP_LLO_SCHEDULER": True, "XLA_TPU_RESCHEDULE_DMA_DONES": True},
        ),
    )(qt, kt, vt)
    return jnp.swapaxes(ot.reshape(B, H, D, Sq), 2, 3)
```

```python
import math

import jax
import jax.numpy as jnp
from jax import lax
import jax.experimental.pallas as pl
import jax.experimental.pallas.tpu as pltpu


@jax.jit
def pallas_standalone__mha_softmax__near_ridge_kernel(
    q: jax.Array,
    k: jax.Array,
    v: jax.Array,
):
    B, H, Sq, D = q.shape
    Sk = k.shape[2]
    NH = B * H
    G = 32
    NB = 4
    NG = NH // G
    NT = Sq // 128
    QL = Sq - NT * 128
    assert NH % G == 0 and G % NB == 0 and NT == 3 and QL % 16 == 0 and Sk == 512
    c = (D ** -0.5) * math.log2(math.e)
    dn_t = (((0,), (0,)), ((), ()))
    dn_nt = (((1,), (1,)), ((), ()))

    NCH, NSTEP, LEADS = 8, 24, (420, 400, 360)
    CCH, CSTEP, CLEAD = 7, 20, 400
    LAT, DR, TAIL0, MAX_AT = 125, 16, -140, -50

    qt = jnp.swapaxes(q, 2, 3).reshape(NH, D, Sq)
    kt = jnp.swapaxes(k, 2, 3).reshape(NH, D, Sk)
    vt = jnp.swapaxes(v, 2, 3).reshape(NH, D, Sk)

    def kernel(q_hbm, k_hbm, v_hbm, o_hbm, qb, kb, vb, ob, sq, sk, sv, so):
        def cp_in(src, h, dst, sem, slot):
            return pltpu.make_async_copy(src.at[h], dst.at[slot], sem.at[slot])

        def cp_out(h, slot):
            return pltpu.make_async_copy(ob.at[slot], o_hbm.at[h], so.at[slot])

        cp_in(k_hbm, 0, kb, sk, 0).start()
        cp_in(q_hbm, 0, qb, sq, 0).start()
        for s in range(1, NB):
            cp_in(k_hbm, s, kb, sk, s).start()
            cp_in(q_hbm, s, qb, sq, s).start()
            cp_in(v_hbm, s - 1, vb, sv, s - 1).start()
        cp_in(v_hbm, NB - 1, vb, sv, NB - 1).start()

        def body(g, carry):
            base = g * G
            zero = lax.shift_right_logical(g, 24)
            not_first = g > 0
            not_last = g < NG - 1

            def dep(x8, anchor):
                a = pltpu.bitcast(anchor, jnp.int32) & jnp.full(x8.shape, zero, jnp.int32)
                return pltpu.bitcast(pltpu.bitcast(x8, jnp.int32) | a, jnp.float32)

            def pad128(av):
                return av if av.shape[1] == 128 else jnp.pad(av, ((0, 0), (0, 128 - av.shape[1])))

            def waits_qk(j):
                s = j % NB
                cp_in(k_hbm, 0, kb, sk, s).wait()
                cp_in(q_hbm, 0, qb, sq, s).wait()

            def waits_vo(j):
                s = j % NB
                cp_in(v_hbm, 0, vb, sv, s).wait()
                if j >= NB:
                    cp_out(0, s).wait()
                else:
                    @pl.when(not_first)
                    def _():
                        cp_out(0, s).wait()

            def maybe(j, f):
                if j + NB < G:
                    f()
                else:
                    pl.when(not_last)(f)

            def start_kq(j):
                s = j % NB

                def f():
                    cp_in(k_hbm, base + j + NB, kb, sk, s).start()
                    cp_in(q_hbm, base + j + NB, qb, sq, s).start()
                maybe(j, f)

            def qk(j):
                s = j % NB
                kk = kb[s]
                qq = qb[s]
                sc = lax.dot_general(qq[:, 384:Sq], kk, dn_t, preferred_element_type=jnp.float32)
                sb1 = lax.dot_general(kk[:, 0:256], qq[:, 256:384], dn_t, preferred_element_type=jnp.float32)
                sb2 = lax.dot_general(kk[:, 256:512], qq[:, 256:384], dn_t, preferred_element_type=jnp.float32)
                sa = lax.dot_general(kk, qq[:, 0:256], dn_t, preferred_element_type=jnp.float32)
                if j == 0:
                    start_kq(j)
                return sa, jnp.concatenate([sb1, sb2], axis=0), sc

            def pick(t_want, nxt, prev, outs):
                cands = []
                if nxt is not None:
                    t_c, t_b, t_a = -(2 * QL + 256 + 512), -(256 + 512), -512
                    cands += [(t_c + LAT + 8 * i, ("C1", i)) for i in range(QL // 8)]
                    cands += [(t_c + QL + LAT + 8 * i, ("C2", i)) for i in range(QL // 8)]
                    cands += [(t_b + LAT + 8 * i, ("B", i)) for i in range(Sk // 16)]
                    cands += [(t_a + LAT + 8 * i, ("A", i)) for i in range(Sk // 8)]
                elif prev is not None:
                    for n in range(NT + 1):
                        cands += [(D * (n - 4) + LAT + 8 * i, ("p", n, i)) for i in range(D // 8)]
                for n in range(len(outs)):
                    cands += [(D * n + LAT + 8 * i, ("o", n, i)) for i in range(D // 8)]
                if not cands:
                    return None
                w = min(cands, key=lambda x: abs(x[0] - t_want))[1]
                if w[0] == "A":
                    return nxt[0][8 * w[1]:8 * w[1] + 8, 128:256]
                if w[0] == "B":
                    return nxt[1][8 * w[1]:8 * w[1] + 8, :]
                if w[0] == "C1":
                    return nxt[2][8 * w[1]:8 * w[1] + 8, 0:128]
                if w[0] == "C2":
                    return nxt[2][8 * w[1]:8 * w[1] + 8, 384:512]
                if w[0] == "p":
                    return pad128(prev[w[1]][8 * w[2]:8 * w[2] + 8, :])
                return pad128(outs[w[1]][8 * w[2]:8 * w[2] + 8, :])

            def softmax_rows(sc, max_anchor, anchors):
                pm = sc[:, 0:128]
                for a in range(128, Sk, 128):
                    pm = jnp.maximum(pm, sc[:, a:a + 128])
                if max_anchor is not None:
                    pm = pm.reshape(QL // 8, 8, 128)
                    pm = dep(pm, jnp.broadcast_to(max_anchor[None], pm.shape)).reshape(QL, 128)
                mc = jnp.max(pm, axis=1, keepdims=True)
                rows = QL // CCH
                ps = []
                for i in range(CCH):
                    r, r2 = i * rows, (i + 1) * rows
                    x = sc[r:r2] - mc[r:r2]
                    if anchors[i] is not None:
                        cd = dep(jnp.full((8, 128), c, jnp.float32), anchors[i])
                        cd4 = jnp.concatenate([cd] * (Sk // 128), axis=1)
                        x = (x.reshape(rows // 8, 8, Sk) * cd4[None]).reshape(rows, Sk)
                    else:
                        x = x * c
                    p = jnp.exp2(x)
                    l = jnp.sum(p, axis=1, keepdims=True)
                    inv = pl.reciprocal(l, approx=True)
                    inv = inv * (2.0 - l * inv)
                    ps.append(p * inv)
                return jnp.concatenate(ps, axis=0).astype(jnp.bfloat16)

            def sm_pv(j, cur, nxt, prev):
                s = j % NB
                sta, stb, sc = cur
                vv = vb[s]
                outs = []
                rows = Sk // NCH
                for n in range(NT):
                    st = sta[:, n * 128:(n + 1) * 128] if n < 2 else stb
                    m8 = jnp.broadcast_to(jnp.max(st, axis=0, keepdims=True), (8, 128))
                    ps = []
                    lacc = None
                    for i in range(NCH):
                        lead = LEADS[n] + (TAIL0 if (nxt is None and n == 0) else 0)
                        av = pick(D * n - lead + i * NSTEP, nxt, prev, outs)
                        mi = m8 if av is None else dep(m8, av)
                        x = st[i * rows:(i + 1) * rows].reshape(rows // 8, 8, 128) - mi[None]
                        p = jnp.exp2(x * c)
                        ls = jnp.sum(p, axis=0)
                        lacc = ls if lacc is None else lacc + ls
                        ps.append(p.reshape(rows, 128))
                    l = jnp.sum(lacc, axis=0, keepdims=True)
                    ot = jnp.dot(vv, jnp.concatenate(ps, axis=0).astype(jnp.bfloat16),
                                 preferred_element_type=jnp.float32)
                    outs.append(ot)
                    ob[s, :, n * 128:(n + 1) * 128] = (ot * (1.0 / l)).astype(ob.dtype)
                if j == G - 1:
                    pltpu.make_async_copy(ob.at[s, :, 0:NT * 128], o_hbm.at[base + j, :, 0:NT * 128],
                                          so.at[s]).start()
                anchors = [pick(D * NT - CLEAD + i * CSTEP, nxt, prev, outs) for i in range(CCH)]
                plast = softmax_rows(sc, pick(MAX_AT, nxt, prev, outs), anchors)
                ot = lax.dot_general(vv, plast, dn_nt, preferred_element_type=jnp.float32)
                outs.append(ot)
                ob[s, :, NT * 128:Sq] = ot.astype(ob.dtype)

                av16 = outs[2][DR:DR + 16, :].astype(jnp.bfloat16)
                vb[s, 0:16, 0:128] = av16
                if j + 1 < G:
                    kb[(j + 1) % NB, 0:16, 0:128] = av16
                    qb[(j + 1) % NB, 0:16, 0:128] = av16
                    start_kq(j + 1)
                maybe(j, lambda: cp_in(v_hbm, base + j + NB, vb, sv, s).start())
                if j == G - 1:
                    pltpu.make_async_copy(ob.at[s, :, NT * 128:Sq], o_hbm.at[base + j, :, NT * 128:Sq],
                                          so.at[s]).start()
                else:
                    cp_out(base + j, s).start()
                if j + 2 < G:
                    waits_qk(j + 2)
                if j + 1 < G:
                    waits_vo(j + 1)
                return outs

            waits_qk(0)
            s_next = qk(0)
            waits_qk(1)
            waits_vo(0)
            prev = None
            for j in range(G):
                cur = s_next
                s_next = qk(j + 1) if j + 1 < G else None
                prev = sm_pv(j, cur, s_next, prev)
            return carry

        lax.fori_loop(0, NG, body, 0)
        for s in range(NB):
            cp_out(0, s).wait()

    ot = pl.pallas_call(
        kernel,
        grid=(1,),
        in_specs=[pl.BlockSpec(memory_space=pl.ANY)] * 3,
        out_specs=pl.BlockSpec(memory_space=pl.ANY),
        out_shape=jax.ShapeDtypeStruct((NH, D, Sq), q.dtype),
        scratch_shapes=[
            pltpu.VMEM((NB, D, Sq), q.dtype),
            pltpu.VMEM((NB, D, Sk), k.dtype),
            pltpu.VMEM((NB, D, Sk), v.dtype),
            pltpu.VMEM((NB, D, Sq), q.dtype),
            pltpu.SemaphoreType.DMA((NB,)),
            pltpu.SemaphoreType.DMA((NB,)),
            pltpu.SemaphoreType.DMA((NB,)),
            pltpu.SemaphoreType.DMA((NB,)),
        ],
        compiler_params=pltpu.CompilerParams(
            dimension_semantics=("arbitrary",),
            vmem_limit_bytes=64 * 1024 * 1024,
            flags={"XLA_TPU_RESCHEDULE_DMA_DONES": True},
        ),
    )(qt, kt, vt)
    return jnp.swapaxes(ot.reshape(B, H, D, Sq), 2, 3)
```
